```python
import os as _os
_os.environ.setdefault("JAX_PLATFORMS", "cpu")
import jax
import jax.numpy as jnp

def _softmax(x, axis=-1):
    return jax.nn.softmax(x, axis=axis)
def _gelu(x):
    return jax.nn.gelu(x, approximate=True)
def _silu(x):
    return jax.nn.silu(x)
def _sigmoid(x):
    return jax.nn.sigmoid(x)
def _layernorm(x, axis=-1, eps=1e-5):
    m = jnp.mean(x, axis=axis, keepdims=True)
    v = jnp.var(x, axis=axis, keepdims=True)
    return (x - m) / jnp.sqrt(v + eps)
def _scatter_add(tgt, idx, src, axis=0):
    return tgt.at[idx].add(src)
def _segment_sum(src, seg, n):
    return jax.ops.segment_sum(src, seg, n)
class _Rng:
    def __init__(self, key):
        self._k = key
    def _next(self):
        self._k, sub = jax.random.split(self._k)
        return sub
    def normal(self, shape):
        return jax.random.normal(self._next(), shape, dtype=jnp.bfloat16)
    def randint(self, lo, hi, shape):
        return jax.random.randint(self._next(), shape, lo, hi, dtype=jnp.int32)
    def uniform(self, shape, lo=0.0, hi=1.0):
        return jax.random.uniform(self._next(), shape, jnp.bfloat16, lo, hi)
    def permutation(self, n):
        return jax.random.permutation(self._next(), n)


kernel_name = 'standalone__grn__sampling'

def setup_inputs():
    _rng = _Rng(jax.random.key(int.from_bytes(__import__("os").urandom(4), "little")))
    _w = (lambda a: (lambda t: t.astype(jnp.bfloat16) if jnp.issubdtype(t.dtype, jnp.floating) else t)(jnp.asarray(a)))
    B, S, D = 512, 32, 640
    return {
        "x": _w((lambda *s: _rng.normal(s) * 0.05)(B, S, D)),
        "g": _w((lambda *s: _rng.normal(s) * 0.1)(D) * 0.1),
        "b": _w((lambda *s: _rng.normal(s) * 0.1)(D) * 0.1),
    }

def reference(x, g, b):
    gx = jnp.sqrt((x * x).sum(axis=-2, keepdims=True))
    nx = gx / (gx.mean(axis=-1, keepdims=True) + 1e-6)
    return g * (x * nx) + b + x
```

```python
import jax
import jax.numpy as jnp
import jax.experimental.pallas as pl
import jax.experimental.pallas.tpu as pltpu

_R = 8
_TAIL = 1
_PRE = 2


def _grn(x, g, b):
    xf = x.astype(jnp.float32)
    gx = jnp.sqrt(jnp.sum(xf * xf, axis=-2, keepdims=True))
    inv = 1.0 / (jnp.mean(gx, axis=-1, keepdims=True) + 1e-6)
    return (xf * (g * (gx * inv) + 1.0) + b).astype(x.dtype)


def _grn_kernel(x_hbm, g_hbm, b_hbm, o_hbm, buf, g_vmem, b_vmem, sems):
    regions, n = buf.shape[0], buf.shape[1]
    half = n // 2

    def cols(ref, start, size):
        return ref.at[:, pl.ds(start, size)]

    def read(start, size, k):
        return pltpu.make_async_copy(
            cols(x_hbm, start, size), cols(buf, start, size), sems.at[k])

    def write(i):
        return pltpu.make_async_copy(cols(buf, i, 1), cols(o_hbm, i, 1), sems.at[3])

    read_a = read(0, half, 0)
    read_b = read(half, n - half - _TAIL, 1)
    read_c = read(n - _TAIL, _TAIL, 2)
    read_g = pltpu.make_async_copy(g_hbm, g_vmem, sems.at[0])
    read_bias = pltpu.make_async_copy(b_hbm, b_vmem, sems.at[0])
    read_a.start()
    read_g.start()
    read_bias.start()
    read_b.start()
    read_c.start()

    read_a.wait()
    read_g.wait()
    read_bias.wait()
    g = g_vmem[...].astype(jnp.float32).reshape(1, -1)
    b = b_vmem[...].astype(jnp.float32).reshape(1, -1)

    def compute(i):
        for r in range(regions):
            buf[r, i] = _grn(buf[r, i], g, b)

    @pl.loop(0, half)
    def _(i):
        compute(i)

    read_b.wait()
    for i in range(_PRE):
        write(i).start()
    read_c.wait()

    @pl.loop(0, n - half)
    def _(i):
        compute(half + i)
        write(_PRE + i).start()

    @pl.loop(_PRE + n - half, n)
    def _(i):
        write(i).start()

    pltpu.make_async_copy(buf, o_hbm, sems.at[3]).wait()


@jax.jit
def pallas_standalone__grn__sampling_kernel(x: jax.Array, g: jax.Array, b: jax.Array):
    B, S, D = x.shape
    shape = (_R, B // _R, S, D)
    out = pl.pallas_call(
        _grn_kernel,
        in_specs=[pl.BlockSpec(memory_space=pl.ANY)] * 3,
        out_specs=pl.BlockSpec(memory_space=pl.ANY),
        out_shape=jax.ShapeDtypeStruct(shape, x.dtype),
        scratch_shapes=[
            pltpu.VMEM(shape, x.dtype),
            pltpu.VMEM((D,), g.dtype),
            pltpu.VMEM((D,), b.dtype),
            pltpu.SemaphoreType.DMA((4,)),
        ],
        compiler_params=pltpu.CompilerParams(vmem_limit_bytes=64 * 2**20),
    )(x.reshape(shape), g, b)
    return out.reshape(B, S, D)
```

```python
import functools

import jax
import jax.numpy as jnp
import jax.experimental.pallas as pl
import jax.experimental.pallas.tpu as pltpu

_EPS = 1e-6
_PIECE_ROWS = 16
_STREAMS = 8
_FIRST_STRIDE = 77
_GROUP = 8
_LEAD_ROUNDS = 3
_ROUNDS_PER_GROUP = 2


def _grn(x, g, b):
    xf = x.astype(jnp.float32)
    sum_sq = jnp.sum(jnp.sum(xf * xf, axis=0), axis=0, keepdims=True)
    gx = jnp.sqrt(sum_sq)
    nx = gx * (1.0 / (jnp.mean(gx, axis=-1, keepdims=True) + _EPS))
    return (xf * (g * nx + 1.0) + b).astype(x.dtype)


def _grn_kernel(x_hbm, g_hbm, b_hbm, o_hbm, buf, g_vmem, b_vmem, write_sem, *,
                pieces_per_elem):
    n_pieces = buf.shape[0]
    group_pieces = _GROUP * pieces_per_elem
    n_groups = n_pieces // group_pieces

    second_base = _STREAMS * _FIRST_STRIDE
    second_stride = n_pieces // _STREAMS - _FIRST_STRIDE
    early = pl.cdiv(second_base, group_pieces)
    overlapped_rounds = _LEAD_ROUNDS + (n_groups - early) * _ROUNDS_PER_GROUP
    assert n_pieces % group_pieces == 0 and n_pieces % _STREAMS == 0
    assert second_stride > 0 and 2 <= early < n_groups - 1
    assert overlapped_rounds <= _FIRST_STRIDE

    def write_round(base, stride, i):
        for stream in range(_STREAMS):
            piece = pl.ds(base + stream * stride + i, 1)
            pltpu.make_async_copy(buf.at[piece], o_hbm.at[piece], write_sem).start()

    write_first = functools.partial(write_round, 0, _FIRST_STRIDE)
    write_second = functools.partial(write_round, second_base, second_stride)

    def read_and_compute(sems):
        edges = (0, (early + 1) // 2, early, n_groups - 1, n_groups)
        reads = []
        for k, (lo, hi) in enumerate(zip(edges[:-1], edges[1:])):
            span = pl.ds(lo * group_pieces, (hi - lo) * group_pieces)
            reads.append(
                pltpu.make_async_copy(x_hbm.at[span], buf.at[span], sems.at[k]))
        read_g = pltpu.make_async_copy(g_hbm, g_vmem, sems.at[0])
        read_b = pltpu.make_async_copy(b_hbm, b_vmem, sems.at[0])

        for copy in (reads[0], read_g, read_b, *reads[1:]):
            copy.start()
        for copy in (reads[0], read_g, read_b):
            copy.wait()
        g = g_vmem[...].astype(jnp.float32).reshape(1, -1)
        b = b_vmem[...].astype(jnp.float32).reshape(1, -1)

        def compute(group):
            for e in range(_GROUP):
                elem = pl.ds((group * _GROUP + e) * pieces_per_elem, pieces_per_elem)
                buf[elem] = _grn(buf[elem], g, b)

        @pl.loop(0, early)
        def _(group):
            pl.when(group == edges[1])(reads[1].wait)
            compute(group)

        reads[2].wait()
        for i in range(_LEAD_ROUNDS):
            write_first(i)

        @pl.loop(early, n_groups)
        def _(group):
            pl.when(group == edges[3])(reads[3].wait)
            compute(group)
            for t in range(_ROUNDS_PER_GROUP):
                write_first(_LEAD_ROUNDS + (group - early) * _ROUNDS_PER_GROUP + t)

    pl.run_scoped(read_and_compute, pltpu.SemaphoreType.DMA((4,)))

    pl.loop(overlapped_rounds, _FIRST_STRIDE)(write_first)
    pl.loop(0, second_stride)(write_second)
    pltpu.make_async_copy(buf, o_hbm, write_sem).wait()


@jax.jit
def pallas_standalone__grn__sampling_kernel(x: jax.Array, g: jax.Array, b: jax.Array):
    B, S, D = x.shape
    assert S % _PIECE_ROWS == 0
    pieces_per_elem = S // _PIECE_ROWS
    shape = (B * pieces_per_elem, _PIECE_ROWS, D)
    out = pl.pallas_call(
        functools.partial(_grn_kernel, pieces_per_elem=pieces_per_elem),
        in_specs=[pl.BlockSpec(memory_space=pl.ANY)] * 3,
        out_specs=pl.BlockSpec(memory_space=pl.ANY),
        out_shape=jax.ShapeDtypeStruct(shape, x.dtype),
        scratch_shapes=[
            pltpu.VMEM(shape, x.dtype),
            pltpu.VMEM((D,), g.dtype),
            pltpu.VMEM((D,), b.dtype),
            pltpu.SemaphoreType.DMA,
        ],
        compiler_params=pltpu.CompilerParams(vmem_limit_bytes=48 * 2**20),
    )(x.reshape(shape), g, b)
    return out.reshape(B, S, D)
```
